```python
import os as _os
_os.environ.setdefault("JAX_PLATFORMS", "cpu")
import jax
import jax.numpy as jnp

def _softmax(x, axis=-1):
    return jax.nn.softmax(x, axis=axis)
def _gelu(x):
    return jax.nn.gelu(x, approximate=True)
def _silu(x):
    return jax.nn.silu(x)
def _sigmoid(x):
    return jax.nn.sigmoid(x)
def _layernorm(x, axis=-1, eps=1e-5):
    m = jnp.mean(x, axis=axis, keepdims=True)
    v = jnp.var(x, axis=axis, keepdims=True)
    return (x - m) / jnp.sqrt(v + eps)
def _scatter_add(tgt, idx, src, axis=0):
    return tgt.at[idx].add(src)
def _segment_sum(src, seg, n):
    return jax.ops.segment_sum(src, seg, n)
class _Rng:
    def __init__(self, key):
        self._k = key
    def _next(self):
        self._k, sub = jax.random.split(self._k)
        return sub
    def normal(self, shape):
        return jax.random.normal(self._next(), shape, dtype=jnp.bfloat16)
    def randint(self, lo, hi, shape):
        return jax.random.randint(self._next(), shape, lo, hi, dtype=jnp.int32)
    def uniform(self, shape, lo=0.0, hi=1.0):
        return jax.random.uniform(self._next(), shape, jnp.bfloat16, lo, hi)
    def permutation(self, n):
        return jax.random.permutation(self._next(), n)


kernel_name = 'sequential_preLN__softmax_full_mha__glu_gated_swiglu__prompt'

def setup_inputs():
    _rng = _Rng(jax.random.key(int.from_bytes(__import__("os").urandom(4), "little")))
    _w = (lambda a: (lambda t: t.astype(jnp.bfloat16) if jnp.issubdtype(t.dtype, jnp.floating) else t)(jnp.asarray(a)))
    def _A_setup():
        B, S, D = 1, 2048, 640
        return {
            "x": _w((lambda *s: _rng.normal(s) * 0.05)(B, S, D)),
            "wqkv": _w((lambda *s: _rng.normal(s) * 0.05)(D, 3 * D)),
            "wo": _w((lambda *s: _rng.normal(s) * 0.05)(D, D)),
        }
    _A_in = _A_setup()

    def _B_setup():
        B, S, D, F = 1, 2048, 640, 1728
        return {
            "x": _w((lambda *s: _rng.normal(s) * 0.05)(B, S, D)),
            "w1": _w((lambda *s: _rng.normal(s) * 0.05)(D, F) * (2.0 / D) ** 0.5),
            "w3": _w((lambda *s: _rng.normal(s) * 0.05)(D, F) * (2.0 / D) ** 0.5),
            "w2": _w((lambda *s: _rng.normal(s) * 0.05)(F, D) * (2.0 / F) ** 0.5),
        }
    _B_in = _B_setup()

    return {
        "A_x": _A_in["x"],
        "A_wqkv": _A_in["wqkv"],
        "A_wo": _A_in["wo"],
        "B_x": _B_in["x"],
        "B_w1": _B_in["w1"],
        "B_w3": _B_in["w3"],
        "B_w2": _B_in["w2"],
    }

def reference(A_x, A_wqkv, A_wo, B_x, B_w1, B_w3, B_w2):
    def _A_ref(x, wqkv, wo):
        B, S, D = x.shape
        H = 32; Dh = D // H
        qkv = (lambda x, *d: x.transpose(*d))((x @ wqkv).reshape(B, S, 3, H, Dh), 2, 0, 3, 1, 4)
        q, k, v = qkv[0], qkv[1], qkv[2]
        scale = Dh ** -0.5
        scores = jnp.einsum("bhqd,bhkd->bhqk", q, k) * scale
        p = _softmax(scores, axis=-1)
        o = jnp.einsum("bhqk,bhkd->bhqd", p, v)
        return (lambda x, *d: x.transpose(*d))(o, 0, 2, 1, 3).reshape(B, S, D) @ wo

    def _B_ref(x, w1, w3, w2):
        gate = jnp.einsum("bsd,df->bsf", x, w1)
        up = jnp.einsum("bsd,df->bsf", x, w3)
        h = _silu(gate) * up
        out = jnp.einsum("bsf,fd->bsd", h, w2)
        return out

    x = A_x
    h = x + _A_ref(_layernorm(x, axis=-1), A_wqkv, A_wo)
    h2 = h + _B_ref(_layernorm(h, axis=-1), B_w1, B_w3, B_w2)
    return h2
```

```python
import functools

import jax
import jax.numpy as jnp
import jax.experimental.pallas as pl
import jax.experimental.pallas.tpu as pltpu

S = 2048
D = 640
H = 32
DH = 20
F = 1728
HP = 32
HPG = 128 // HP
NG = H // HPG
DP = H * HP
EPS = 1e-5
LOG2E = 1.4426950408889634

BM = 256


def _layernorm_f32(x):
    mu = jnp.mean(x, axis=-1, keepdims=True)
    xc = x - mu
    var = jnp.mean(xc * xc, axis=-1, keepdims=True)
    return xc * jax.lax.rsqrt(var + EPS)


def _kernel(x_ref, wq_ref, wkt_ref, wv_ref, wo_ref, w1_ref, w3_ref, w2_ref,
            o_ref, xn_ref, kt_ref, v_ref):
    i = pl.program_id(0)

    @pl.when(i == 0)
    def _():
        xn = _layernorm_f32(x_ref[...].astype(jnp.float32)).astype(jnp.bfloat16)
        xn_ref[...] = xn
        kt = jax.lax.dot_general(wkt_ref[...], xn, (((1,), (1,)), ((), ())),
                                 preferred_element_type=jnp.float32)
        kt_ref[...] = kt.astype(jnp.bfloat16)
        v = jnp.dot(xn, wv_ref[...], preferred_element_type=jnp.float32)
        lane = jax.lax.broadcasted_iota(jnp.int32, (S, DP), 1)
        v = jnp.where(lane % HP == DH, 1.0, v)
        v_ref[...] = v.astype(jnp.bfloat16)

    row0 = pl.multiple_of(i * BM, BM)
    xn_blk = xn_ref[pl.ds(row0, BM), :]
    scale = (DH ** -0.5) * LOG2E
    q = jnp.dot(xn_blk, wq_ref[...], preferred_element_type=jnp.float32) * scale

    lane128 = jax.lax.broadcasted_iota(jnp.int32, (1, 128), 1)
    outs = []
    for g in range(NG):
        qg = q[:, g * 128:(g + 1) * 128]
        qs = jnp.concatenate(
            [jnp.where(lane128 // HP == j, qg, 0.0) for j in range(HPG)], axis=0
        ).astype(jnp.bfloat16)
        s = jnp.dot(qs, kt_ref[g * 128:(g + 1) * 128, :],
                    preferred_element_type=jnp.float32)
        m = jnp.max(s, axis=-1, keepdims=True)
        p = jnp.exp2(s - m).astype(jnp.bfloat16)
        os_ = jnp.dot(p, v_ref[:, g * 128:(g + 1) * 128],
                      preferred_element_type=jnp.float32)
        og = jnp.zeros((BM, 128), jnp.float32)
        for j in range(HPG):
            oj = os_[j * BM:(j + 1) * BM, :]
            l = jnp.sum(jnp.where(lane128 == j * HP + DH, oj, 0.0), axis=-1, keepdims=True)
            og = og + jnp.where(lane128 // HP == j, oj / l, 0.0)
        outs.append(og.astype(jnp.bfloat16))
    o = jnp.concatenate(outs, axis=1)
    attn = jnp.dot(o, wo_ref[...], preferred_element_type=jnp.float32)
    h = x_ref[pl.ds(row0, BM), :].astype(jnp.float32) + attn

    hn = _layernorm_f32(h).astype(jnp.bfloat16)
    gate = jnp.dot(hn, w1_ref[...], preferred_element_type=jnp.float32)
    up = jnp.dot(hn, w3_ref[...], preferred_element_type=jnp.float32)
    act = (gate * jax.nn.sigmoid(gate) * up).astype(jnp.bfloat16)
    out = h + jnp.dot(act, w2_ref[...], preferred_element_type=jnp.float32)
    o_ref[...] = out.astype(o_ref.dtype)


def _pad_heads(w):
    w = w.reshape(D, H, DH)
    w = jnp.pad(w, ((0, 0), (0, 0), (0, HP - DH)))
    return w.reshape(D, DP)


@jax.jit
def pallas_sequential_preLN__softmax_full_mha__glu_gated_swiglu__prompt_kernel(
    A_x: jax.Array,
    A_wqkv: jax.Array,
    A_wo: jax.Array,
    B_x: jax.Array,
    B_w1: jax.Array,
    B_w3: jax.Array,
    B_w2: jax.Array,
):
    x = A_x.reshape(S, D)
    wq = _pad_heads(A_wqkv[:, :D])
    wkt = _pad_heads(A_wqkv[:, D:2 * D]).T
    wv = _pad_heads(A_wqkv[:, 2 * D:])
    wo = jnp.pad(A_wo.reshape(H, DH, D), ((0, 0), (0, HP - DH), (0, 0))).reshape(DP, D)

    def full(shape):
        return pl.BlockSpec(shape, lambda i: (0,) * len(shape))

    out = pl.pallas_call(
        _kernel,
        grid=(S // BM,),
        in_specs=[
            full((S, D)), full((D, DP)), full((DP, D)), full((D, DP)), full((DP, D)),
            full((D, F)), full((D, F)), full((F, D)),
        ],
        out_specs=pl.BlockSpec((BM, D), lambda i: (i, 0)),
        out_shape=jax.ShapeDtypeStruct((S, D), jnp.bfloat16),
        scratch_shapes=[
            pltpu.VMEM((S, D), jnp.bfloat16),
            pltpu.VMEM((DP, S), jnp.bfloat16),
            pltpu.VMEM((S, DP), jnp.bfloat16),
        ],
        compiler_params=pltpu.CompilerParams(
            dimension_semantics=("arbitrary",),
            vmem_limit_bytes=100 * 1024 * 1024,
        ),
    )(x, wq, wkt, wv, wo, B_w1, B_w3, B_w2)
    return out.reshape(1, S, D)
```

```python
import functools
import jax
import jax.numpy as jnp
import jax.experimental.pallas as pl
import jax.experimental.pallas.tpu as pltpu

S = 2048; D = 640; H = 32; DH = 20; F = 1728
HP = 32; HPG = 128 // HP; NG = H // HPG; DP = H * HP
EPS = 1e-5
LOG2E = 1.4426950408889634
BM = 128
R = 128
CPH = BM // R
NC = H * CPH
NT = (((1,), (1,)), ((), ()))
TN = (((0,), (0,)), ((), ()))


def _layernorm_f32(x):
    mu = jnp.mean(x, axis=-1, keepdims=True)
    xc = x - mu
    var = jnp.mean(xc * xc, axis=-1, keepdims=True)
    return xc * jax.lax.rsqrt(var + EPS)


def _kernel(x_ref, wq_ref, wkt_ref, wvt_ref, wo_ref, w1_ref, w3_ref, w2_ref,
            o_ref, xn_ref, kt_ref, vt_ref, qm_ref, ot_ref, sa_ref, sb_ref):
    i = pl.program_id(0)

    @pl.when(i == 0)
    def _():
        xn = _layernorm_f32(x_ref[...].astype(jnp.float32)).astype(jnp.bfloat16)
        xn_ref[...] = xn
        row = jax.lax.broadcasted_iota(jnp.int32, (128, S), 0)
        for g in range(NG):
            kt = jax.lax.dot_general(wkt_ref[g * 128:(g + 1) * 128, :], xn, NT,
                                     preferred_element_type=jnp.float32)
            kt_ref[g] = kt.astype(jnp.bfloat16)
            vt = jax.lax.dot_general(wvt_ref[g * 128:(g + 1) * 128, :], xn, NT,
                                     preferred_element_type=jnp.float32)
            vt = jnp.where(row % HP == DH, 1.0, vt)
            vt_ref[g * 128:(g + 1) * 128, :] = vt.astype(jnp.bfloat16)

    row0 = pl.multiple_of(i * BM, BM)
    xn_blk = xn_ref[pl.ds(row0, BM), :]
    scale = (DH ** -0.5) * LOG2E
    q = jnp.dot(xn_blk, wq_ref[...], preferred_element_type=jnp.float32) * scale
    lane128 = jax.lax.broadcasted_iota(jnp.int32, (1, 128), 1)
    for g in range(NG):
        qg = q[:, g * 128:(g + 1) * 128]
        for j in range(HPG):
            qm_ref[g * HPG + j] = jnp.where(lane128 // HP == j, qg, 0.0).astype(jnp.bfloat16)

    def qk(c):
        h = c // CPH
        rc = c % CPH
        qm = qm_ref[h, pl.ds(pl.multiple_of(rc * R, R), R), :]
        s = jnp.dot(qm, kt_ref[h // HPG], preferred_element_type=jnp.float32)
        return s, jnp.max(s, axis=-1, keepdims=True)

    def soft_pv(c, s, m):
        h = c // CPH
        rc = c % CPH
        p = jnp.exp2(s - m).astype(jnp.bfloat16)
        hr = pl.multiple_of(h * HP, HP)
        ot = jax.lax.dot_general(vt_ref[pl.ds(hr, HP), :], p, NT,
                                 preferred_element_type=jnp.float32)
        ot_ref[rc, pl.ds(hr, HP), :] = ot

    s, ma = qk(0)
    sa_ref[...] = s

    def body(k, ma):
        c = 2 * k
        s, mb = qk(c + 1)
        sb_ref[...] = s
        soft_pv(c, sa_ref[...], ma)
        s, ma = qk(jnp.minimum(c + 2, NC - 1))
        sa_ref[...] = s
        soft_pv(c + 1, sb_ref[...], mb)
        return ma

    jax.lax.fori_loop(0, NC // 2, body, ma, unroll=4)

    attn = []
    for rc in range(CPH):
        ot = ot_ref[rc].reshape(H, HP, R)
        ot = (ot / ot[:, DH:DH + 1, :]).reshape(DP, R)
        attn.append(jax.lax.dot_general(ot.astype(jnp.bfloat16), wo_ref[...], TN,
                                        preferred_element_type=jnp.float32))
    h = x_ref[pl.ds(row0, BM), :].astype(jnp.float32) + jnp.concatenate(attn, axis=0)

    hn = _layernorm_f32(h).astype(jnp.bfloat16)
    gate = jnp.dot(hn, w1_ref[...], preferred_element_type=jnp.float32)
    up = jnp.dot(hn, w3_ref[...], preferred_element_type=jnp.float32)
    act = (gate * jax.nn.sigmoid(gate) * up).astype(jnp.bfloat16)
    out = h + jnp.dot(act, w2_ref[...], preferred_element_type=jnp.float32)
    o_ref[...] = out.astype(o_ref.dtype)


def _pad_heads(w):
    w = w.reshape(D, H, DH)
    w = jnp.pad(w, ((0, 0), (0, 0), (0, HP - DH)))
    return w.reshape(D, DP)


@jax.jit
def pallas_sequential_preLN__softmax_full_mha__glu_gated_swiglu__prompt_kernel(
    A_x, A_wqkv, A_wo, B_x, B_w1, B_w3, B_w2):
    x = A_x.reshape(S, D)
    wq = _pad_heads(A_wqkv[:, :D])
    wkt = _pad_heads(A_wqkv[:, D:2 * D]).T
    wvt = _pad_heads(A_wqkv[:, 2 * D:]).T
    wo = jnp.pad(A_wo.reshape(H, DH, D), ((0, 0), (0, HP - DH), (0, 0))).reshape(DP, D)

    def full(shape):
        return pl.BlockSpec(shape, lambda i: (0,) * len(shape))

    out = pl.pallas_call(
        _kernel,
        grid=(S // BM,),
        in_specs=[
            full((S, D)), full((D, DP)), full((DP, D)), full((DP, D)), full((DP, D)),
            full((D, F)), full((D, F)), full((F, D)),
        ],
        out_specs=pl.BlockSpec((BM, D), lambda i: (i, 0)),
        out_shape=jax.ShapeDtypeStruct((S, D), jnp.bfloat16),
        scratch_shapes=[
            pltpu.VMEM((S, D), jnp.bfloat16),
            pltpu.VMEM((NG, 128, S), jnp.bfloat16),
            pltpu.VMEM((DP, S), jnp.bfloat16),
            pltpu.VMEM((H, BM, 128), jnp.bfloat16),
            pltpu.VMEM((CPH, DP, R), jnp.float32),
            pltpu.VMEM((R, S), jnp.float32),
            pltpu.VMEM((R, S), jnp.float32),
        ],
        compiler_params=pltpu.CompilerParams(
            dimension_semantics=("arbitrary",),
            vmem_limit_bytes=100 * 1024 * 1024,
        ),
    )(x, wq, wkt, wvt, wo, B_w1, B_w3, B_w2)
    return out.reshape(1, S, D)
```

```python
import functools
import jax
import jax.numpy as jnp
import jax.experimental.pallas as pl
import jax.experimental.pallas.tpu as pltpu

S = 2048; D = 640; H = 32; DH = 20; F = 1728
HP = 32; DP = H * HP
EPS = 1e-5
LOG2E = 1.4426950408889634
BM = 128
R = 128
UNROLL = 5
NC = H
NT = (((1,), (1,)), ((), ()))
TN = (((0,), (0,)), ((), ()))
TT = (((0,), (1,)), ((), ()))


def _win(h):
    lo = DH * h
    base = (lo // 128) * 128
    return base + 64 if lo - base + DH > 128 else base


def _layernorm_f32(x):
    mu = jnp.mean(x, axis=-1, keepdims=True)
    xc = x - mu
    var = jnp.mean(xc * xc, axis=-1, keepdims=True)
    return xc * jax.lax.rsqrt(var + EPS)


def _kernel(x_ref, w_ref, wo_hbm, w1_hbm, w3_hbm, w2_hbm,
            o_ref, xn_ref, kt_ref, vt32_ref, vt_ref, qm_ref, ot_ref, sa_ref, sb_ref,
            wo_ref, w1_ref, w3_ref, w2_ref, sems):
    i = pl.program_id(0)

    def _copies():
        return [pltpu.make_async_copy(src, dst, sems.at[n]) for n, (src, dst) in enumerate(
            ((wo_hbm, wo_ref), (w1_hbm, w1_ref), (w3_hbm, w3_ref), (w2_hbm, w2_ref)))]

    @pl.when(i == 0)
    def _():
        for cp in _copies():
            cp.start()

    @pl.when(i == 0)
    def _():
        xn = _layernorm_f32(x_ref[...].astype(jnp.float32)).astype(jnp.bfloat16)
        xn_ref[...] = xn
        for g in range(D // 128):
            kt = jax.lax.dot_general(w_ref[:, D + g * 128:D + (g + 1) * 128], xn, TT,
                                     preferred_element_type=jnp.float32)
            kt_ref[g * 128:(g + 1) * 128, :] = kt.astype(jnp.bfloat16)
        row = jax.lax.broadcasted_iota(jnp.int32, (DP, S), 0)
        vt32_ref[...] = jnp.where(row % HP == DH, 1.0, 0.0)
        for g in range(D // 128):
            vt = jax.lax.dot_general(w_ref[:, 2 * D + g * 128:2 * D + (g + 1) * 128], xn, TT,
                                     preferred_element_type=jnp.float32)
            for h in range(H):
                lo, hi = max(DH * h, 128 * g), min(DH * h + DH, 128 * (g + 1))
                if lo < hi:
                    vt32_ref[HP * h + lo - DH * h:HP * h + hi - DH * h, :] = vt[lo - 128 * g:hi - 128 * g, :]
        vt_ref[...] = vt32_ref[...].astype(jnp.bfloat16)

    row0 = pl.multiple_of(i * BM, BM)
    xn_blk = xn_ref[pl.ds(row0, BM), :]
    scale = (DH ** -0.5) * LOG2E
    q = jnp.dot(xn_blk, w_ref[:, :D], preferred_element_type=jnp.float32) * scale
    lane128 = jax.lax.broadcasted_iota(jnp.int32, (1, 128), 1)
    for h in range(H):
        w0 = _win(h)
        a = DH * h - w0
        qw = q[:, w0:w0 + 128]
        qm_ref[h] = jnp.where((lane128 >= a) & (lane128 < a + DH), qw, 0.0).astype(jnp.bfloat16)

    def qk(h):
        lo = DH * h
        base = (lo // 128) * 128
        w0 = pl.multiple_of(jnp.where(lo - base + DH > 128, base + 64, base), 64)
        s = jnp.dot(qm_ref[h], kt_ref[pl.ds(w0, 128), :], preferred_element_type=jnp.float32)
        return s, jnp.max(s, axis=-1, keepdims=True)

    def soft_pv(h, s, m):
        p = jnp.exp2(s - m).astype(jnp.bfloat16)
        hr = pl.multiple_of(h * HP, HP)
        ot_ref[pl.ds(hr, HP), :] = jax.lax.dot_general(vt_ref[pl.ds(hr, HP), :], p, NT,
                                                       preferred_element_type=jnp.float32)

    s, ma = qk(0)
    sa_ref[...] = s

    def body(k, ma):
        c = 2 * k
        s, mb = qk(c + 1)
        sb_ref[...] = s
        soft_pv(c, sa_ref[...], ma)
        s, ma = qk(c + 2)
        sa_ref[...] = s
        soft_pv(c + 1, sb_ref[...], mb)
        return ma

    ma = jax.lax.fori_loop(0, NC // 2 - 1, body, ma, unroll=UNROLL)
    c = NC - 2
    s, mb = qk(c + 1)
    sb_ref[...] = s
    soft_pv(c, sa_ref[...], ma)
    soft_pv(c + 1, sb_ref[...], mb)

    @pl.when(i == 0)
    def _():
        for cp in _copies():
            cp.wait()

    ot = ot_ref[...].reshape(H, HP, R)
    ot = (ot / ot[:, DH:DH + 1, :]).reshape(DP, R)
    attn = jax.lax.dot_general(ot.astype(jnp.bfloat16), wo_ref[...], TN,
                               preferred_element_type=jnp.float32)
    h = x_ref[pl.ds(row0, BM), :].astype(jnp.float32) + attn

    hn = _layernorm_f32(h).astype(jnp.bfloat16)
    gate = jax.lax.dot_general(hn, w1_ref[...], NT, preferred_element_type=jnp.float32)
    up = jax.lax.dot_general(hn, w3_ref[...], NT, preferred_element_type=jnp.float32)
    act = (gate * jax.nn.sigmoid(gate) * up).astype(jnp.bfloat16)
    out = h + jnp.dot(act, w2_ref[...], preferred_element_type=jnp.float32)
    o_ref[...] = out.astype(o_ref.dtype)


@jax.jit
def pallas_sequential_preLN__softmax_full_mha__glu_gated_swiglu__prompt_kernel(
    A_x, A_wqkv, A_wo, B_x, B_w1, B_w3, B_w2):
    x = A_x.reshape(S, D)
    wo = jnp.pad(A_wo.reshape(H, DH, D), ((0, 0), (0, HP - DH), (0, 0))).reshape(DP, D)

    def full(shape):
        return pl.BlockSpec(shape, lambda i: (0,) * len(shape))

    out = pl.pallas_call(
        _kernel,
        grid=(S // BM,),
        in_specs=[
            full((S, D)), full((D, 3 * D)),
            pl.BlockSpec(memory_space=pl.ANY), pl.BlockSpec(memory_space=pl.ANY),
            pl.BlockSpec(memory_space=pl.ANY), pl.BlockSpec(memory_space=pl.ANY),
        ],
        out_specs=pl.BlockSpec((BM, D), lambda i: (i, 0)),
        out_shape=jax.ShapeDtypeStruct((S, D), jnp.bfloat16),
        scratch_shapes=[
            pltpu.VMEM((S, D), jnp.bfloat16),
            pltpu.VMEM((D, S), jnp.bfloat16),
            pltpu.VMEM((DP, S), jnp.float32),
            pltpu.VMEM((DP, S), jnp.bfloat16),
            pltpu.VMEM((H, BM, 128), jnp.bfloat16),
            pltpu.VMEM((DP, R), jnp.float32),
            pltpu.VMEM((R, S), jnp.float32),
            pltpu.VMEM((R, S), jnp.float32),
            pltpu.VMEM((DP, D), jnp.bfloat16),
            pltpu.VMEM((F, D), jnp.bfloat16),
            pltpu.VMEM((F, D), jnp.bfloat16),
            pltpu.VMEM((F, D), jnp.bfloat16),
            pltpu.SemaphoreType.DMA((4,)),
        ],
        compiler_params=pltpu.CompilerParams(
            dimension_semantics=("arbitrary",),
            vmem_limit_bytes=100 * 1024 * 1024,
        ),
    )(x, A_wqkv, wo, B_w1.T, B_w3.T, B_w2)
    return out.reshape(1, S, D)
```
